```python
import os as _os
_os.environ.setdefault("JAX_PLATFORMS", "cpu")
import jax
import jax.numpy as jnp

def _softmax(x, axis=-1):
    return jax.nn.softmax(x, axis=axis)
def _gelu(x):
    return jax.nn.gelu(x, approximate=True)
def _silu(x):
    return jax.nn.silu(x)
def _sigmoid(x):
    return jax.nn.sigmoid(x)
def _layernorm(x, axis=-1, eps=1e-5):
    m = jnp.mean(x, axis=axis, keepdims=True)
    v = jnp.var(x, axis=axis, keepdims=True)
    return (x - m) / jnp.sqrt(v + eps)
def _scatter_add(tgt, idx, src, axis=0):
    return tgt.at[idx].add(src)
def _segment_sum(src, seg, n):
    return jax.ops.segment_sum(src, seg, n)
class _Rng:
    def __init__(self, key):
        self._k = key
    def _next(self):
        self._k, sub = jax.random.split(self._k)
        return sub
    def normal(self, shape):
        return jax.random.normal(self._next(), shape, dtype=jnp.bfloat16)
    def randint(self, lo, hi, shape):
        return jax.random.randint(self._next(), shape, lo, hi, dtype=jnp.int32)
    def uniform(self, shape, lo=0.0, hi=1.0):
        return jax.random.uniform(self._next(), shape, jnp.bfloat16, lo, hi)
    def permutation(self, n):
        return jax.random.permutation(self._next(), n)


kernel_name = 'concat_heads__sliding_block_cached__sliding_block_cached__decode'

def setup_inputs():
    _rng = _Rng(jax.random.key(int.from_bytes(__import__("os").urandom(4), "little")))
    _w = (lambda a: (lambda t: t.astype(jnp.bfloat16) if jnp.issubdtype(t.dtype, jnp.floating) else t)(jnp.asarray(a)))
    def _A_setup():
        B, Sq, D = 1, 1, 512
        Hq, Hkv, Sk, Dh = 32, 32, 32768, 128
        assert Hq % Hkv == 0, (Hq, Hkv)
        return {
            "x": _w((lambda *s: _rng.normal(s) * 0.8)(B, Sq, D)),
            "k_cache": _w((lambda *s: _rng.normal(s) * 0.8)(B, Hkv, Sk, Dh)),
            "v_cache": _w((lambda *s: _rng.normal(s) * 0.05)(B, Hkv, Sk, Dh)),
            "wq": _w((lambda *s: _rng.normal(s) * 0.8)(D, Hq * Dh) * (D ** -0.5)),
            "wo": _w((lambda *s: _rng.normal(s) * 0.05)(Hq * Dh, D) * ((Hq * Dh) ** -0.5)),
        }
    _A_in = _A_setup()

    def _B_setup():
        B, Sq, D = 1, 1, 512
        Hq, Hkv, Sk, Dh = 32, 32, 32768, 128
        assert Hq % Hkv == 0, (Hq, Hkv)
        return {
            "x": _w((lambda *s: _rng.normal(s) * 0.8)(B, Sq, D)),
            "k_cache": _w((lambda *s: _rng.normal(s) * 0.8)(B, Hkv, Sk, Dh)),
            "v_cache": _w((lambda *s: _rng.normal(s) * 0.05)(B, Hkv, Sk, Dh)),
            "wq": _w((lambda *s: _rng.normal(s) * 0.8)(D, Hq * Dh) * (D ** -0.5)),
            "wo": _w((lambda *s: _rng.normal(s) * 0.05)(Hq * Dh, D) * ((Hq * Dh) ** -0.5)),
        }
    _B_in = _B_setup()

    return {
        "A_x": _A_in["x"],
        "A_k_cache": _A_in["k_cache"],
        "A_v_cache": _A_in["v_cache"],
        "A_wq": _A_in["wq"],
        "A_wo": _A_in["wo"],
        "B_x": _B_in["x"],
        "B_k_cache": _B_in["k_cache"],
        "B_v_cache": _B_in["v_cache"],
        "B_wq": _B_in["wq"],
        "B_wo": _B_in["wo"],
    }

def reference(A_x, A_k_cache, A_v_cache, A_wq, A_wo, B_x, B_k_cache, B_v_cache, B_wq, B_wo):
    def _A_ref(x, k_cache, v_cache, wq, wo):
        B, Sq, D = x.shape
        Hq, Dh = 32, 128
        Hkv, Sk = k_cache.shape[1], k_cache.shape[2]
        W = min(4096, max(256, Sk // 4))
        rep = Hq // Hkv
        q = (lambda x, *d: x.transpose(*d))((x @ wq).reshape(B, Sq, Hq, Dh), 0, 2, 1, 3)
        k = jnp.repeat(k_cache[:, :, Sk - W:, :], rep, axis=1)
        v = jnp.repeat(v_cache[:, :, Sk - W:, :], rep, axis=1)
        scores = jnp.einsum("bhqd,bhkd->bhqk", q, k) * (Dh ** -0.5)
        p = _softmax(scores, axis=-1)
        o = jnp.einsum("bhqk,bhkd->bhqd", p, v)
        return (lambda x, *d: x.transpose(*d))(o, 0, 2, 1, 3).reshape(B, Sq, Hq * Dh) @ wo

    def _B_ref(x, k_cache, v_cache, wq, wo):
        B, Sq, D = x.shape
        Hq, Dh = 32, 128
        Hkv, Sk = k_cache.shape[1], k_cache.shape[2]
        W = min(4096, max(256, Sk // 4))
        rep = Hq // Hkv
        q = (lambda x, *d: x.transpose(*d))((x @ wq).reshape(B, Sq, Hq, Dh), 0, 2, 1, 3)
        k = jnp.repeat(k_cache[:, :, Sk - W:, :], rep, axis=1)
        v = jnp.repeat(v_cache[:, :, Sk - W:, :], rep, axis=1)
        scores = jnp.einsum("bhqd,bhkd->bhqk", q, k) * (Dh ** -0.5)
        p = _softmax(scores, axis=-1)
        o = jnp.einsum("bhqk,bhkd->bhqd", p, v)
        return (lambda x, *d: x.transpose(*d))(o, 0, 2, 1, 3).reshape(B, Sq, Hq * Dh) @ wo

    a = _A_ref(A_x, A_k_cache, A_v_cache, A_wq, A_wo)
    b = _B_ref(B_x, B_k_cache, B_v_cache, B_wq, B_wo)
    return jnp.concatenate([a, b], axis=-1)
```

```python
import functools
import jax
import jax.numpy as jnp
from jax import lax
import jax.experimental.pallas as pl
import jax.experimental.pallas.tpu as pltpu

H, DH, W, D = 32, 128, 4096, 512
HG = 4
NG = H // HG
UR = 512
NCH = W // UR
PR = 32
NS = 3
NWQ = 4
NWO = 4
NKV = NG * NCH
F32 = jnp.float32
BF16 = jnp.bfloat16


def kernel(ax, ak, av, awq, awo, bx, bk, bv, bwq, bwo, o_ref,
           kv, wqb, wob, xb, q8s, lhs, sem, xsem):
    Sk = ak.shape[2]
    w0 = Sk - W

    def issue_wq(i):
        s = sem.at[i % NS]
        def body(t, c):
            r = pl.multiple_of((t // 4) * 16, 16)
            cc = pl.multiple_of((t % 4) * 1024, 1024)
            pltpu.make_async_copy(awq.at[pl.ds(i * 128 + r, 16), pl.ds(cc, 1024)],
                                  wqb.at[i, 0, pl.ds(r, 16), pl.ds(cc, 1024)], s).start(priority=0)
            pltpu.make_async_copy(bwq.at[pl.ds(i * 128 + r, 16), pl.ds(cc, 1024)],
                                  wqb.at[i, 1, pl.ds(r, 16), pl.ds(cc, 1024)], s).start(priority=1)
            return c
        lax.fori_loop(0, 32, body, 0)

    def issue_kv(u, slot):
        g = u // NCH
        c = u % NCH
        h0 = g * HG
        s = sem.at[slot]
        def body(t, carry):
            r = pl.multiple_of(t * PR, PR)
            rs = pl.multiple_of(w0 + c * UR + r, PR)
            for j, (src, p) in enumerate(((ak, 0), (av, 1), (bk, 0), (bv, 1))):
                pltpu.make_async_copy(src.at[0, pl.ds(h0, HG), pl.ds(rs, PR), :],
                                      kv.at[slot, j, :, pl.ds(r, PR), :], s).start(priority=p)
            return carry
        lax.fori_loop(0, UR // PR, body, 0)

    def issue_wo(i, slot):
        s = sem.at[slot]
        def body(t, c):
            r = pl.multiple_of(t * 32, 32)
            rs = pl.multiple_of(i * 1024 + r, 32)
            pltpu.make_async_copy(awo.at[pl.ds(rs, 32), :], wob.at[i, 0, pl.ds(r, 32), :], s).start(priority=0)
            pltpu.make_async_copy(bwo.at[pl.ds(rs, 32), :], wob.at[i, 1, pl.ds(r, 32), :], s).start(priority=1)
            return c
        lax.fori_loop(0, 32, body, 0)

    xa_cp = pltpu.make_async_copy(ax, xb.at[0], xsem.at[0])
    xb_cp = pltpu.make_async_copy(bx, xb.at[1], xsem.at[0])
    xa_cp.start()
    xb_cp.start()
    for i in range(NS):
        issue_wq(i)
    xa_cp.wait()
    xb_cp.wait()
    xA = jnp.broadcast_to(xb[0, 0], (8, D))
    xB = jnp.broadcast_to(xb[1, 0], (8, D))

    row = lax.broadcasted_iota(jnp.int32, (8, DH), 0)

    qA = jnp.zeros((8, H * DH), F32)
    qB = jnp.zeros((8, H * DH), F32)
    for i in range(NWQ):
        pltpu.make_async_copy(wqb.at[i], wqb.at[i], sem.at[i % NS]).wait()
        qA = qA + jnp.dot(xA[:, i * 128:(i + 1) * 128], wqb[i, 0], preferred_element_type=F32)
        qB = qB + jnp.dot(xB[:, i * 128:(i + 1) * 128], wqb[i, 1], preferred_element_type=F32)
        n = i + NS
        if n < NWQ:
            issue_wq(n)
        else:
            issue_kv(n - NWQ, n % NS)
    for g in range(NG):
        q8 = jnp.zeros((8, DH), F32)
        for j in range(HG):
            h = g * HG + j
            q8 = jnp.where(row == j, qA[:, h * DH:(h + 1) * DH], q8)
            q8 = jnp.where(row == HG + j, qB[:, h * DH:(h + 1) * DH], q8)
        q8s[g] = q8

    rowS = lax.broadcasted_iota(jnp.int32, (8, UR), 0)
    scale = DH ** -0.5

    def kv_body(u, carry):
        m, l, acc = carry
        g = u // NCH
        c = u % NCH
        slot = (u + NWQ) % NS
        first = c == 0
        m = jnp.where(first, -jnp.inf, m)
        l = jnp.where(first, 0.0, l)
        acc = jnp.where(first, 0.0, acc)
        pltpu.make_async_copy(kv.at[slot], kv.at[slot], sem.at[slot]).wait()
        q8 = q8s[g].astype(BF16)
        s = jnp.zeros((8, UR), F32)
        for b in range(2):
            for j in range(HG):
                sj = lax.dot_general(q8, kv[slot, 2 * b, j], (((1,), (1,)), ((), ())),
                                     preferred_element_type=F32)
                s = jnp.where(rowS == b * HG + j, sj, s)
        s = s * scale
        m_new = jnp.maximum(m, jnp.max(s, axis=-1, keepdims=True))
        alpha = jnp.exp(m - m_new)
        p = jnp.exp(s - m_new)
        l = l * alpha + jnp.sum(p, axis=-1, keepdims=True)
        pb = p.astype(BF16)
        o = jnp.zeros((8, DH), F32)
        for b in range(2):
            for j in range(HG):
                oj = jnp.dot(pb, kv[slot, 2 * b + 1, j], preferred_element_type=F32)
                o = jnp.where(row == b * HG + j, oj, o)
        acc = acc * alpha + o

        @pl.when(c == NCH - 1)
        def _():
            o8 = acc / l
            for b in range(2):
                for j in range(HG):
                    lhs[b, g, :, j * DH:(j + 1) * DH] = jnp.where(row == b * HG + j, o8, 0.0)

        n = u + NS
        @pl.when(n < NKV)
        def _():
            issue_kv(n, slot)
        @pl.when(n >= NKV)
        def _():
            issue_wo(n - NKV, slot)
        return m_new, l, acc

    init = (jnp.full((8, 1), -jnp.inf, F32), jnp.zeros((8, 1), F32), jnp.zeros((8, DH), F32))
    lax.fori_loop(0, NKV, kv_body, init)

    accA = jnp.zeros((8, D), F32)
    accB = jnp.zeros((8, D), F32)
    for i in range(NWO):
        slot = (NWQ + NKV + i) % NS
        pltpu.make_async_copy(wob.at[i], wob.at[i], sem.at[slot]).wait()
        if i + NS < NWO:
            issue_wo(i + NS, slot)
        for gg in range(2):
            g = 2 * i + gg
            accA = accA + jnp.dot(lhs[0, g].astype(BF16), wob[i, 0, gg * 512:(gg + 1) * 512, :], preferred_element_type=F32)
            accB = accB + jnp.dot(lhs[1, g].astype(BF16), wob[i, 1, gg * 512:(gg + 1) * 512, :], preferred_element_type=F32)
    o_ref[0, :, 0:D] = jnp.sum(accA, axis=0, keepdims=True).astype(o_ref.dtype)
    o_ref[0, :, D:2 * D] = jnp.sum(accB, axis=0, keepdims=True).astype(o_ref.dtype)


@jax.jit
def pallas_concat_heads__sliding_block_cached__sliding_block_cached__decode_kernel(
        A_x, A_k_cache, A_v_cache, A_wq, A_wo, B_x, B_k_cache, B_v_cache, B_wq, B_wo):
    anyspec = pl.BlockSpec(memory_space=pl.ANY)
    return pl.pallas_call(
        kernel,
        in_specs=[anyspec] * 10,
        out_specs=pl.BlockSpec(memory_space=pltpu.VMEM),
        out_shape=jax.ShapeDtypeStruct((1, 1, 2 * D), BF16),
        scratch_shapes=[
            pltpu.VMEM((NS, 4, HG, UR, DH), BF16),
            pltpu.VMEM((NWQ, 2, 128, H * DH), BF16),
            pltpu.VMEM((NWO, 2, 1024, D), BF16),
            pltpu.VMEM((2, 1, 1, D), BF16),
            pltpu.VMEM((NG, 8, DH), F32),
            pltpu.VMEM((2, NG, 8, HG * DH), F32),
            pltpu.SemaphoreType.DMA((NS,)),
            pltpu.SemaphoreType.DMA((1,)),
        ],
        compiler_params=pltpu.CompilerParams(vmem_limit_bytes=64 * 1024 * 1024),
    )(A_x, A_k_cache, A_v_cache, A_wq, A_wo, B_x, B_k_cache, B_v_cache, B_wq, B_wo)
```

```python
import jax
import jax.numpy as jnp
from jax import lax
import jax.experimental.pallas as pl
import jax.experimental.pallas.tpu as pltpu

F32 = jnp.float32
BF16 = jnp.bfloat16

H, DH, D = 32, 128, 512
HG = 4
NG = H // HG
GW = HG * DH
UR = 512
PR = 32
NS = 3
NSLAB = 4
START_P1 = 12
TAIL_ROWS = 32
MXU_PIECES = ((0, 2), (2, 3))
VPU_PIECES = ((0, 96), (96, 128))


def _kernel(ax, ak, av, awq, awo, bx, bk, bv, bwq, bwo, o_ref,
            kv, wqb, wob, xb, q8s, lhs, sem, wsem, *, window):
    w0 = ak.shape[2] - window
    nch = window // UR
    nkv = NG * nch
    wq_steps = (D // NSLAB // 8) * NG
    blk_steps = DH // 8

    def wq_cp(b, t):
        r = pl.multiple_of((t // NG) * 8, 8)
        g = t % NG
        cc = pl.multiple_of(g * GW, GW)
        return pltpu.make_async_copy(
            (awq, bwq)[b].at[:, pl.ds(r, 8), pl.ds(cc, GW)],
            wqb.at[g, b, :, pl.ds(r, 8), :], wsem.at[0])

    def wo_cp(b, t, s):
        r = pl.multiple_of((t % blk_steps) * 8, 8)
        rs = pl.multiple_of(t * 8, 8)
        return pltpu.make_async_copy(
            (awo, bwo)[b].at[:, pl.ds(rs, 8), :],
            wob.at[t // blk_steps, b, :, pl.ds(r, 8), :], s)

    def issue_wq():
        for t in range(START_P1):
            for b in range(2):
                wq_cp(b, t).start(priority=1)

        def body(t, carry):
            for b in range(2):
                wq_cp(b, t).start(priority=b)
            return carry
        lax.fori_loop(START_P1, wq_steps, body, 0)

    def issue_kv(u, slot):
        h0 = (u // nch) * HG
        r0 = w0 + (u % nch) * UR

        def body(t, carry):
            r = pl.multiple_of(t * PR, PR)
            rs = pl.multiple_of(r0 + r, PR)
            for j, src in enumerate((ak, av, bk, bv)):
                pltpu.make_async_copy(
                    src.at[0, pl.ds(h0, HG), pl.ds(rs, PR), :],
                    kv.at[slot, j, :, pl.ds(r, PR), :],
                    sem.at[slot]).start(priority=j % 2)
            return carry
        lax.fori_loop(0, UR // PR, body, 0)

    def issue_wo(t0, n, sa, sb):
        def body(t, carry):
            wo_cp(0, t0 + t, sa).start(priority=0)
            wo_cp(1, t0 + t, sb).start(priority=1)
            return carry
        lax.fori_loop(0, n, body, 0)

    def wait_ref(ref, s):
        pltpu.make_async_copy(ref, ref, s).wait()

    xa_cp = pltpu.make_async_copy(ax, xb.at[0], wsem.at[0])
    xb_cp = pltpu.make_async_copy(bx, xb.at[1], wsem.at[0])
    xa_cp.start()
    xb_cp.start()
    issue_wq()
    for i in range(NS):
        issue_kv(i, i)
    xa_cp.wait()
    xb_cp.wait()
    wait_ref(wqb, wsem.at[0])

    row = lax.broadcasted_iota(jnp.int32, (8, DH), 0)
    row_s = lax.broadcasted_iota(jnp.int32, (8, UR), 0)
    scale = DH ** -0.5

    def kv_body(u, carry):
        m, l, acc = carry
        g = u // nch
        c = u % nch
        slot = u % NS
        first = c == 0

        @pl.when(first)
        def _():
            q8 = jnp.zeros((8, DH), F32)
            for b in range(2):
                x8 = jnp.broadcast_to(xb[b, 0], (8, D))
                qg = jnp.dot(x8, wqb[g, b].reshape(D, GW), preferred_element_type=F32)
                for j in range(HG):
                    q8 = jnp.where(row == b * HG + j, qg[:, j * DH:(j + 1) * DH], q8)
            q8s[...] = q8

        m = jnp.where(first, -jnp.inf, m)
        l = jnp.where(first, 0.0, l)
        acc = jnp.where(first, 0.0, acc)
        wait_ref(kv.at[slot], sem.at[slot])
        q8 = q8s[...].astype(BF16)
        s = jnp.zeros((8, UR), F32)
        for b in range(2):
            for j in range(HG):
                sj = lax.dot_general(q8, kv[slot, 2 * b, j], (((1,), (1,)), ((), ())),
                                     preferred_element_type=F32)
                s = jnp.where(row_s == b * HG + j, sj, s)
        s = s * scale
        m_new = jnp.maximum(m, jnp.max(s, axis=-1, keepdims=True))
        alpha = jnp.exp(m - m_new)
        p = jnp.exp(s - m_new)
        l = l * alpha + jnp.sum(p, axis=-1, keepdims=True)
        pb = p.astype(BF16)
        o = jnp.zeros((8, DH), F32)
        for b in range(2):
            for j in range(HG):
                oj = jnp.dot(pb, kv[slot, 2 * b + 1, j], preferred_element_type=F32)
                o = jnp.where(row == b * HG + j, oj, o)
        acc = acc * alpha + o

        @pl.when(c == nch - 1)
        def _():
            lhs[g] = acc / l

        n = u + NS

        @pl.when(n < nkv)
        def _():
            issue_kv(n, slot)

        @pl.when(n >= nkv)
        def _():
            issue_wo((n - nkv) * 2 * blk_steps, 2 * blk_steps, sem.at[slot], sem.at[slot])
        return m_new, l, acc

    init = (jnp.full((8, 1), -jnp.inf, F32), jnp.zeros((8, 1), F32),
            jnp.zeros((8, DH), F32))
    lax.fori_loop(0, nkv, kv_body, init)

    last = 7
    issue_wo(6 * blk_steps, blk_steps, wsem.at[0], wsem.at[1])

    def b_sem(sl, r):
        for i, (lo, hi) in enumerate(MXU_PIECES):
            if lo <= sl < hi:
                return wsem.at[2 + i]
        for i, (lo, hi) in enumerate(VPU_PIECES):
            if lo <= r < hi:
                return wsem.at[2 + len(MXU_PIECES) + i]

    for sl in range(NSLAB):
        for r in range(0, DH, TAIL_ROWS):
            for b in range(2):
                pltpu.make_async_copy(
                    (awo, bwo)[b].at[sl, pl.ds(last * DH + r, TAIL_ROWS), :],
                    wob.at[last, b, sl, pl.ds(r, TAIL_ROWS), :],
                    b_sem(sl, r) if b else wsem.at[0]).start(priority=b)

    def proj(b, blk, slabs):
        res = None
        for sl in slabs:
            h = sl * 8 + blk
            o_h = jnp.where(row == b * HG + h % HG, lhs[h // HG], 0.0).astype(BF16)
            t = jnp.dot(o_h, wob[blk, b, sl], preferred_element_type=F32)
            res = t if res is None else res + t
        return res

    o_last = lhs[NG - 1][7:8, :].astype(BF16).astype(F32)
    o_col = jnp.broadcast_to(o_last, (DH, DH)).T

    acc_a = jnp.zeros((8, D), F32)
    acc_b = jnp.zeros((8, D), F32)
    for blk in range(6):
        if blk % 2 == 0:
            wait_ref(wob.at[pl.ds(blk, 2)], sem.at[(nkv + blk // 2) % NS])
        acc_a = acc_a + proj(0, blk, range(NSLAB))
        acc_b = acc_b + proj(1, blk, range(NSLAB))
    wait_ref(wob.at[6, 0], wsem.at[0])
    wait_ref(wob.at[last, 0], wsem.at[0])
    acc_a = acc_a + proj(0, 6, range(NSLAB)) + proj(0, last, range(NSLAB))
    o_ref[0, :, 0:D] = jnp.sum(acc_a, axis=0, keepdims=True).astype(o_ref.dtype)
    wait_ref(wob.at[6, 1], wsem.at[1])
    acc_b = acc_b + proj(1, 6, range(NSLAB))
    for i, (lo, hi) in enumerate(MXU_PIECES):
        wait_ref(wob.at[last, 1, pl.ds(lo, hi - lo)], wsem.at[2 + i])
        acc_b = acc_b + proj(1, last, range(lo, hi))
    for i, (lo, hi) in enumerate(VPU_PIECES):
        wait_ref(wob.at[last, 1, NSLAB - 1, pl.ds(lo, hi - lo)],
                 wsem.at[2 + len(MXU_PIECES) + i])
        parts = []
        for cb in range(D // DH):
            w = wob[last, 1, NSLAB - 1, lo:hi, cb * DH:(cb + 1) * DH].astype(F32)
            parts.append(jnp.sum((w * o_col[lo:hi]).reshape((hi - lo) // 8, 8, DH), axis=0))
        acc_b = acc_b + jnp.concatenate(parts, axis=1)
    o_ref[0, :, D:2 * D] = jnp.sum(acc_b, axis=0, keepdims=True).astype(o_ref.dtype)


@jax.jit
def pallas_concat_heads__sliding_block_cached__sliding_block_cached__decode_kernel(
    A_x: jax.Array,
    A_k_cache: jax.Array,
    A_v_cache: jax.Array,
    A_wq: jax.Array,
    A_wo: jax.Array,
    B_x: jax.Array,
    B_k_cache: jax.Array,
    B_v_cache: jax.Array,
    B_wq: jax.Array,
    B_wo: jax.Array,
):
    sk = A_k_cache.shape[2]
    window = min(4096, max(256, sk // 4))
    assert A_x.shape == (1, 1, D) and A_k_cache.shape == (1, H, sk, DH)
    assert B_k_cache.shape == A_k_cache.shape
    assert window % UR == 0 and (sk - window) % PR == 0

    def kernel(*refs):
        _kernel(*refs, window=window)

    def slabs(w):
        return w.reshape(NSLAB, w.shape[0] // NSLAB, w.shape[1])

    any_spec = pl.BlockSpec(memory_space=pl.ANY)
    return pl.pallas_call(
        kernel,
        in_specs=[any_spec] * 10,
        out_specs=pl.BlockSpec(memory_space=pltpu.VMEM),
        out_shape=jax.ShapeDtypeStruct((1, 1, 2 * D), A_x.dtype),
        scratch_shapes=[
            pltpu.VMEM((NS, 4, HG, UR, DH), BF16),
            pltpu.VMEM((NG, 2, NSLAB, D // NSLAB, GW), BF16),
            pltpu.VMEM((8, 2, NSLAB, DH, D), BF16),
            pltpu.VMEM((2, 1, 1, D), BF16),
            pltpu.VMEM((8, DH), F32),
            pltpu.VMEM((NG, 8, DH), F32),
            pltpu.SemaphoreType.DMA((NS,)),
            pltpu.SemaphoreType.DMA((2 + len(MXU_PIECES) + len(VPU_PIECES),)),
        ],
        compiler_params=pltpu.CompilerParams(
            vmem_limit_bytes=64 * 1024 * 1024,
            disable_semaphore_checks=True,
            disable_bounds_checks=True,
        ),
    )(A_x, A_k_cache, A_v_cache, slabs(A_wq), slabs(A_wo),
      B_x, B_k_cache, B_v_cache, slabs(B_wq), slabs(B_wo))
```

```python
import jax
import jax.numpy as jnp
from jax import lax
import jax.experimental.pallas as pl
import jax.experimental.pallas.tpu as pltpu

F32 = jnp.float32
BF16 = jnp.bfloat16

H, DH, D = 32, 128, 512
HG = 4
NG = H // HG
GW = HG * DH
UR = 512
PR = 32
V_SPLIT = 2
GB = 4
NS = 3
NSLAB = 4
START_P1 = 12
TAIL_ROWS = 32
MXU_PIECES = ((0, 2), (2, 3))
VPU_PIECES = ((0, 96), (96, 128))


def _kernel(ax, ak, av, awq, awo, bx, bk, bv, bwq, bwo, o_ref,
            kv, wqb, wob, xb, q8s, lhs, sem, wsem, *, window):
    w0 = ak.shape[2] - window
    nch = window // UR
    nkv = NG * nch
    wq_steps = (D // NSLAB // 8) * NG
    blk_steps = DH // 8

    def wq_cp(b, t):
        r = pl.multiple_of((t // NG) * 8, 8)
        g = t % NG
        cc = pl.multiple_of(g * GW, GW)
        return pltpu.make_async_copy(
            (awq, bwq)[b].at[:, pl.ds(r, 8), pl.ds(cc, GW)],
            wqb.at[g, b, :, pl.ds(r, 8), :], wsem.at[0])

    def wo_cp(b, t, s):
        r = pl.multiple_of((t % blk_steps) * 8, 8)
        rs = pl.multiple_of(t * 8, 8)
        return pltpu.make_async_copy(
            (awo, bwo)[b].at[:, pl.ds(rs, 8), :],
            wob.at[t // blk_steps, b, :, pl.ds(r, 8), :], s)

    def issue_wq():
        for t in range(START_P1):
            for b in range(2):
                wq_cp(b, t).start(priority=1)

        def body(t, carry):
            for b in range(2):
                wq_cp(b, t).start(priority=b)
            return carry
        lax.fori_loop(START_P1, wq_steps, body, 0)

    def issue_kv(u, slot):
        g = u // nch
        h0 = (g * HG, ((g + GB) % NG) * HG)
        r0 = w0 + (u % nch) * UR

        def body(t, carry):
            for j in (0, 3, 2, 1):
                n = V_SPLIT if j % 2 else 1
                pr = PR // n
                for z in range(n):
                    r = pl.multiple_of(t * PR + z * pr, pr)
                    rs = pl.multiple_of(r0 + r, pr)
                    pltpu.make_async_copy(
                        (ak, av, bk, bv)[j].at[0, pl.ds(h0[j // 2], HG), pl.ds(rs, pr), :],
                        kv.at[slot, j, :, pl.ds(r, pr), :],
                        sem.at[slot]).start(priority=j % 2)
            return carry
        lax.fori_loop(0, UR // PR, body, 0)

    def issue_wo(t0, n, sa, sb):
        def body(t, carry):
            wo_cp(0, t0 + t, sa).start(priority=0)
            wo_cp(1, t0 + t, sb).start(priority=1)
            return carry
        lax.fori_loop(0, n, body, 0)

    def wait_ref(ref, s):
        pltpu.make_async_copy(ref, ref, s).wait()

    xa_cp = pltpu.make_async_copy(ax, xb.at[0], wsem.at[1])
    xb_cp = pltpu.make_async_copy(bx, xb.at[1], wsem.at[2])
    xa_cp.start()
    xb_cp.start()
    issue_wq()
    for i in range(NS):
        issue_kv(i, i)
    xa_cp.wait()
    xb_cp.wait()
    wait_ref(wqb, wsem.at[0])

    row = lax.broadcasted_iota(jnp.int32, (8, DH), 0)
    row_s = lax.broadcasted_iota(jnp.int32, (8, UR), 0)
    scale = DH ** -0.5

    def kv_body(u, carry):
        m, l, acc = carry
        g = u // nch
        c = u % nch
        slot = u % NS
        first = c == 0

        @pl.when(first)
        def _():
            q8 = jnp.zeros((8, DH), F32)
            for b in range(2):
                x8 = jnp.broadcast_to(xb[b, 0], (8, D))
                wq_g = wqb[(g + b * GB) % NG, b].reshape(D, GW)
                qg = jnp.dot(x8, wq_g, preferred_element_type=F32)
                for j in range(HG):
                    q8 = jnp.where(row == b * HG + j, qg[:, j * DH:(j + 1) * DH], q8)
            q8s[...] = q8

        m = jnp.where(first, -jnp.inf, m)
        l = jnp.where(first, 0.0, l)
        acc = jnp.where(first, 0.0, acc)
        wait_ref(kv.at[slot], sem.at[slot])
        q8 = q8s[...].astype(BF16)
        s = jnp.zeros((8, UR), F32)
        for b in range(2):
            for j in range(HG):
                sj = lax.dot_general(q8, kv[slot, 2 * b, j], (((1,), (1,)), ((), ())),
                                     preferred_element_type=F32)
                s = jnp.where(row_s == b * HG + j, sj, s)
        s = s * scale
        m_new = jnp.maximum(m, jnp.max(s, axis=-1, keepdims=True))
        alpha = jnp.exp(m - m_new)
        p = jnp.exp(s - m_new)
        l = l * alpha + jnp.sum(p, axis=-1, keepdims=True)
        pb = p.astype(BF16)
        o = jnp.zeros((8, DH), F32)
        for b in range(2):
            for j in range(HG):
                oj = jnp.dot(pb, kv[slot, 2 * b + 1, j], preferred_element_type=F32)
                o = jnp.where(row == b * HG + j, oj, o)
        acc = acc * alpha + o

        @pl.when(c == nch - 1)
        def _():
            lhs[g] = acc / l

        n = u + NS

        @pl.when(n < nkv)
        def _():
            issue_kv(n, slot)

        @pl.when(n >= nkv)
        def _():
            issue_wo((n - nkv) * 2 * blk_steps, 2 * blk_steps, sem.at[slot], sem.at[slot])
        return m_new, l, acc

    init = (jnp.full((8, 1), -jnp.inf, F32), jnp.zeros((8, 1), F32),
            jnp.zeros((8, DH), F32))
    lax.fori_loop(0, nkv, kv_body, init)

    last = 7
    issue_wo(6 * blk_steps, blk_steps, wsem.at[0], wsem.at[1])

    def b_sem(sl, r):
        for i, (lo, hi) in enumerate(MXU_PIECES):
            if lo <= sl < hi:
                return wsem.at[2 + i]
        for i, (lo, hi) in enumerate(VPU_PIECES):
            if lo <= r < hi:
                return wsem.at[2 + len(MXU_PIECES) + i]

    for sl in range(NSLAB):
        for r in range(0, DH, TAIL_ROWS):
            for b in range(2):
                pltpu.make_async_copy(
                    (awo, bwo)[b].at[sl, pl.ds(last * DH + r, TAIL_ROWS), :],
                    wob.at[last, b, sl, pl.ds(r, TAIL_ROWS), :],
                    b_sem(sl, r) if b else wsem.at[0]).start(priority=b)

    def proj(b, blk, slabs):
        res = None
        for sl in slabs:
            h = sl * 8 + blk
            o_g = lhs[(h // HG - b * GB) % NG]
            o_h = jnp.where(row == b * HG + h % HG, o_g, 0.0).astype(BF16)
            t = jnp.dot(o_h, wob[blk, b, sl], preferred_element_type=F32)
            res = t if res is None else res + t
        return res

    o_last = lhs[(NG - 1 - GB) % NG][7:8, :].astype(BF16).astype(F32)
    o_col = jnp.broadcast_to(o_last, (DH, DH)).T

    acc_a = jnp.zeros((8, D), F32)
    acc_b = jnp.zeros((8, D), F32)
    for blk in range(6):
        if blk % 2 == 0:
            wait_ref(wob.at[pl.ds(blk, 2)], sem.at[(nkv + blk // 2) % NS])
        acc_a = acc_a + proj(0, blk, range(NSLAB))
        acc_b = acc_b + proj(1, blk, range(NSLAB))
    wait_ref(wob.at[pl.ds(6, 2), 0], wsem.at[0])
    acc_a = acc_a + proj(0, 6, range(NSLAB)) + proj(0, last, range(NSLAB))
    o_ref[0, :, 0:D] = jnp.sum(acc_a, axis=0, keepdims=True).astype(o_ref.dtype)
    wait_ref(wob.at[6, 1], wsem.at[1])
    acc_b = acc_b + proj(1, 6, range(NSLAB))
    for i, (lo, hi) in enumerate(MXU_PIECES):
        wait_ref(wob.at[last, 1, pl.ds(lo, hi - lo)], wsem.at[2 + i])
        acc_b = acc_b + proj(1, last, range(lo, hi))
    for i, (lo, hi) in enumerate(VPU_PIECES):
        wait_ref(wob.at[last, 1, NSLAB - 1, pl.ds(lo, hi - lo)],
                 wsem.at[2 + len(MXU_PIECES) + i])
        parts = []
        for cb in range(D // DH):
            w = wob[last, 1, NSLAB - 1, lo:hi, cb * DH:(cb + 1) * DH].astype(F32)
            parts.append(jnp.sum((w * o_col[lo:hi]).reshape((hi - lo) // 8, 8, DH), axis=0))
        acc_b = acc_b + jnp.concatenate(parts, axis=1)
    o_ref[0, :, D:2 * D] = jnp.sum(acc_b, axis=0, keepdims=True).astype(o_ref.dtype)


@jax.jit
def pallas_concat_heads__sliding_block_cached__sliding_block_cached__decode_kernel(
    A_x: jax.Array,
    A_k_cache: jax.Array,
    A_v_cache: jax.Array,
    A_wq: jax.Array,
    A_wo: jax.Array,
    B_x: jax.Array,
    B_k_cache: jax.Array,
    B_v_cache: jax.Array,
    B_wq: jax.Array,
    B_wo: jax.Array,
):
    sk = A_k_cache.shape[2]
    window = min(4096, max(256, sk // 4))
    assert A_x.shape == (1, 1, D) and A_k_cache.shape == (1, H, sk, DH)
    assert B_k_cache.shape == A_k_cache.shape
    assert window % UR == 0 and (sk - window) % PR == 0

    def kernel(*refs):
        _kernel(*refs, window=window)

    def slabs(w):
        return w.reshape(NSLAB, w.shape[0] // NSLAB, w.shape[1])

    any_spec = pl.BlockSpec(memory_space=pl.ANY)
    return pl.pallas_call(
        kernel,
        in_specs=[any_spec] * 10,
        out_specs=pl.BlockSpec(memory_space=pltpu.VMEM),
        out_shape=jax.ShapeDtypeStruct((1, 1, 2 * D), A_x.dtype),
        scratch_shapes=[
            pltpu.VMEM((NS, 4, HG, UR, DH), BF16),
            pltpu.VMEM((NG, 2, NSLAB, D // NSLAB, GW), BF16),
            pltpu.VMEM((8, 2, NSLAB, DH, D), BF16),
            pltpu.VMEM((2, 1, 1, D), BF16),
            pltpu.VMEM((8, DH), F32),
            pltpu.VMEM((NG, 8, DH), F32),
            pltpu.SemaphoreType.DMA((NS,)),
            pltpu.SemaphoreType.DMA((2 + len(MXU_PIECES) + len(VPU_PIECES),)),
        ],
        compiler_params=pltpu.CompilerParams(
            vmem_limit_bytes=64 * 1024 * 1024,
            disable_semaphore_checks=True,
            disable_bounds_checks=True,
        ),
    )(A_x, A_k_cache, A_v_cache, slabs(A_wq), slabs(A_wo),
      B_x, B_k_cache, B_v_cache, slabs(B_wq), slabs(B_wo))
```

```python
import jax
import jax.numpy as jnp
from jax import lax
import jax.experimental.pallas as pl
import jax.experimental.pallas.tpu as pltpu

F32 = jnp.float32
BF16 = jnp.bfloat16

H, DH, D = 32, 128, 512
HG = 4
NG = H // HG
GW = HG * DH
UR = 512
PR = 32
V_SPLIT = 2
GB = 4
NS = 3
NSLAB = 4
WQ_SPLIT = 2
START_P1 = 6
TAIL_ROWS = 32
MXU_PIECES = ((0, 2), (2, 3))
VPU_PIECES = ((0, 96), (96, 128))


def _kernel(ax, ak, av, awq, awo, bx, bk, bv, bwq, bwo, o_ref,
            kv, wqb, wob, xb, q8s, lhs, sem, wsem, *, window):
    w0 = ak.shape[2] - window
    nch = window // UR
    nkv = NG * nch
    wq_steps = (D // NSLAB // 8) * NG
    blk_steps = DH // 8

    def start_wq(b, t, prio):
        r = pl.multiple_of((t // NG) * 8, 8)
        g = t % NG
        wd = GW // WQ_SPLIT
        for z in range(WQ_SPLIT):
            cc = pl.multiple_of(g * GW + z * wd, wd)
            pltpu.make_async_copy(
                (awq, bwq)[b].at[:, pl.ds(r, 8), pl.ds(cc, wd)],
                wqb.at[g, b, :, pl.ds(r, 8), pl.ds(z * wd, wd)],
                wsem.at[0]).start(priority=prio)

    def wo_cp(b, t, s):
        r = pl.multiple_of((t % blk_steps) * 8, 8)
        rs = pl.multiple_of(t * 8, 8)
        return pltpu.make_async_copy(
            (awo, bwo)[b].at[:, pl.ds(rs, 8), :],
            wob.at[t // blk_steps, b, :, pl.ds(r, 8), :], s)

    def issue_wq():
        for t in range(START_P1):
            for b in range(2):
                start_wq(b, t, 1)

        def body(t, carry):
            for b in range(2):
                start_wq(b, t, b)
            return carry
        lax.fori_loop(START_P1, wq_steps, body, 0)

    def issue_kv(u, slot):
        g = u // nch
        h0 = (g * HG, ((g + GB) % NG) * HG)
        r0 = w0 + (u % nch) * UR

        def body(t, carry):
            for j in (0, 3, 2, 1):
                n = V_SPLIT if j % 2 else 1
                pr = PR // n
                for z in range(n):
                    r = pl.multiple_of(t * PR + z * pr, pr)
                    rs = pl.multiple_of(r0 + r, pr)
                    pltpu.make_async_copy(
                        (ak, av, bk, bv)[j].at[0, pl.ds(h0[j // 2], HG), pl.ds(rs, pr), :],
                        kv.at[slot, j, :, pl.ds(r, pr), :],
                        sem.at[slot]).start(priority=j % 2)
            return carry
        lax.fori_loop(0, UR // PR, body, 0)

    def issue_wo(t0, n, sa, sb):
        def body(t, carry):
            wo_cp(0, t0 + t, sa).start(priority=0)
            wo_cp(1, t0 + t, sb).start(priority=1)
            return carry
        lax.fori_loop(0, n, body, 0)

    def wait_ref(ref, s):
        pltpu.make_async_copy(ref, ref, s).wait()

    xa_cp = pltpu.make_async_copy(ax, xb.at[0], wsem.at[1])
    xb_cp = pltpu.make_async_copy(bx, xb.at[1], wsem.at[2])
    xa_cp.start()
    xb_cp.start()
    issue_wq()
    for i in range(NS):
        issue_kv(i, i)
    xa_cp.wait()
    xb_cp.wait()
    wait_ref(wqb, wsem.at[0])

    row = lax.broadcasted_iota(jnp.int32, (8, DH), 0)
    row_s = lax.broadcasted_iota(jnp.int32, (8, UR), 0)
    scale = DH ** -0.5

    def kv_body(u, carry):
        m, l, acc = carry
        g = u // nch
        c = u % nch
        slot = u % NS
        first = c == 0

        @pl.when(first)
        def _():
            q8 = jnp.zeros((8, DH), F32)
            for b in range(2):
                x8 = jnp.broadcast_to(xb[b, 0], (8, D))
                wq_g = wqb[(g + b * GB) % NG, b].reshape(D, GW)
                qg = jnp.dot(x8, wq_g, preferred_element_type=F32)
                for j in range(HG):
                    q8 = jnp.where(row == b * HG + j, qg[:, j * DH:(j + 1) * DH], q8)
            q8s[...] = q8

        m = jnp.where(first, -jnp.inf, m)
        l = jnp.where(first, 0.0, l)
        acc = jnp.where(first, 0.0, acc)
        wait_ref(kv.at[slot], sem.at[slot])
        q8 = q8s[...].astype(BF16)
        s = jnp.zeros((8, UR), F32)
        for b in range(2):
            for j in range(HG):
                sj = lax.dot_general(q8, kv[slot, 2 * b, j], (((1,), (1,)), ((), ())),
                                     preferred_element_type=F32)
                s = jnp.where(row_s == b * HG + j, sj, s)
        s = s * scale
        m_new = jnp.maximum(m, jnp.max(s, axis=-1, keepdims=True))
        alpha = jnp.exp(m - m_new)
        p = jnp.exp(s - m_new)
        l = l * alpha + jnp.sum(p, axis=-1, keepdims=True)
        pb = p.astype(BF16)
        o = jnp.zeros((8, DH), F32)
        for b in range(2):
            for j in range(HG):
                oj = jnp.dot(pb, kv[slot, 2 * b + 1, j], preferred_element_type=F32)
                o = jnp.where(row == b * HG + j, oj, o)
        acc = acc * alpha + o

        @pl.when(c == nch - 1)
        def _():
            lhs[g] = acc / l

        n = u + NS

        @pl.when(n < nkv)
        def _():
            issue_kv(n, slot)

        @pl.when(n >= nkv)
        def _():
            issue_wo((n - nkv) * 2 * blk_steps, 2 * blk_steps, sem.at[slot], sem.at[slot])
        return m_new, l, acc

    init = (jnp.full((8, 1), -jnp.inf, F32), jnp.zeros((8, 1), F32),
            jnp.zeros((8, DH), F32))
    lax.fori_loop(0, nkv, kv_body, init)

    last = 7
    issue_wo(6 * blk_steps, blk_steps, wsem.at[0], wsem.at[1])

    def b_sem(sl, r):
        for i, (lo, hi) in enumerate(MXU_PIECES):
            if lo <= sl < hi:
                return wsem.at[2 + i]
        for i, (lo, hi) in enumerate(VPU_PIECES):
            if lo <= r < hi:
                return wsem.at[2 + len(MXU_PIECES) + i]

    for sl in range(NSLAB):
        for r in range(0, DH, TAIL_ROWS):
            for b in range(2):
                pltpu.make_async_copy(
                    (awo, bwo)[b].at[sl, pl.ds(last * DH + r, TAIL_ROWS), :],
                    wob.at[last, b, sl, pl.ds(r, TAIL_ROWS), :],
                    b_sem(sl, r) if b else wsem.at[0]).start(priority=b)

    def proj(b, blk, slabs):
        res = None
        for sl in slabs:
            h = sl * 8 + blk
            o_g = lhs[(h // HG - b * GB) % NG]
            o_h = jnp.where(row == b * HG + h % HG, o_g, 0.0).astype(BF16)
            t = jnp.dot(o_h, wob[blk, b, sl], preferred_element_type=F32)
            res = t if res is None else res + t
        return res

    o_last = lhs[(NG - 1 - GB) % NG][7:8, :].astype(BF16).astype(F32)
    o_col = jnp.broadcast_to(o_last, (DH, DH)).T

    acc_a = jnp.zeros((8, D), F32)
    acc_b = jnp.zeros((8, D), F32)
    for blk in range(6):
        if blk % 2 == 0:
            wait_ref(wob.at[pl.ds(blk, 2)], sem.at[(nkv + blk // 2) % NS])
        acc_a = acc_a + proj(0, blk, range(NSLAB))
        acc_b = acc_b + proj(1, blk, range(NSLAB))
    wait_ref(wob.at[pl.ds(6, 2), 0], wsem.at[0])
    acc_a = acc_a + proj(0, 6, range(NSLAB)) + proj(0, last, range(NSLAB))
    o_ref[0, :, 0:D] = jnp.sum(acc_a, axis=0, keepdims=True).astype(o_ref.dtype)
    wait_ref(wob.at[6, 1], wsem.at[1])
    acc_b = acc_b + proj(1, 6, range(NSLAB))
    for i, (lo, hi) in enumerate(MXU_PIECES):
        wait_ref(wob.at[last, 1, pl.ds(lo, hi - lo)], wsem.at[2 + i])
        acc_b = acc_b + proj(1, last, range(lo, hi))
    for i, (lo, hi) in enumerate(VPU_PIECES):
        wait_ref(wob.at[last, 1, NSLAB - 1, pl.ds(lo, hi - lo)],
                 wsem.at[2 + len(MXU_PIECES) + i])
        parts = []
        for cb in range(D // DH):
            w = wob[last, 1, NSLAB - 1, lo:hi, cb * DH:(cb + 1) * DH].astype(F32)
            parts.append(jnp.sum((w * o_col[lo:hi]).reshape((hi - lo) // 8, 8, DH), axis=0))
        acc_b = acc_b + jnp.concatenate(parts, axis=1)
    o_ref[0, :, D:2 * D] = jnp.sum(acc_b, axis=0, keepdims=True).astype(o_ref.dtype)


@jax.jit
def pallas_concat_heads__sliding_block_cached__sliding_block_cached__decode_kernel(
    A_x: jax.Array,
    A_k_cache: jax.Array,
    A_v_cache: jax.Array,
    A_wq: jax.Array,
    A_wo: jax.Array,
    B_x: jax.Array,
    B_k_cache: jax.Array,
    B_v_cache: jax.Array,
    B_wq: jax.Array,
    B_wo: jax.Array,
):
    sk = A_k_cache.shape[2]
    window = min(4096, max(256, sk // 4))
    assert A_x.shape == (1, 1, D) and A_k_cache.shape == (1, H, sk, DH)
    assert B_k_cache.shape == A_k_cache.shape
    assert window % UR == 0 and (sk - window) % PR == 0

    def kernel(*refs):
        _kernel(*refs, window=window)

    def slabs(w):
        return w.reshape(NSLAB, w.shape[0] // NSLAB, w.shape[1])

    any_spec = pl.BlockSpec(memory_space=pl.ANY)
    return pl.pallas_call(
        kernel,
        in_specs=[any_spec] * 10,
        out_specs=pl.BlockSpec(memory_space=pltpu.VMEM),
        out_shape=jax.ShapeDtypeStruct((1, 1, 2 * D), A_x.dtype),
        scratch_shapes=[
            pltpu.VMEM((NS, 4, HG, UR, DH), BF16),
            pltpu.VMEM((NG, 2, NSLAB, D // NSLAB, GW), BF16),
            pltpu.VMEM((8, 2, NSLAB, DH, D), BF16),
            pltpu.VMEM((2, 1, 1, D), BF16),
            pltpu.VMEM((8, DH), F32),
            pltpu.VMEM((NG, 8, DH), F32),
            pltpu.SemaphoreType.DMA((NS,)),
            pltpu.SemaphoreType.DMA((2 + len(MXU_PIECES) + len(VPU_PIECES),)),
        ],
        compiler_params=pltpu.CompilerParams(
            vmem_limit_bytes=64 * 1024 * 1024,
            disable_semaphore_checks=True,
            disable_bounds_checks=True,
        ),
    )(A_x, A_k_cache, A_v_cache, slabs(A_wq), slabs(A_wo),
      B_x, B_k_cache, B_v_cache, slabs(B_wq), slabs(B_wo))
```

```python
import jax
import jax.numpy as jnp
from jax import lax
import jax.experimental.pallas as pl
import jax.experimental.pallas.tpu as pltpu

F32 = jnp.float32
BF16 = jnp.bfloat16

H, DH, D = 32, 128, 512
HG = 4
NG = H // HG
GW = HG * DH
UR = 512
PR = 32
V_SPLIT = 2
GB = 4
BSH = 1
NS = 3
NSLAB = 4
WQ_SPLIT = 2
START_P1 = 6
TAIL_ROWS = 32
MXU_PIECES = ((0, 2), (2, 3))
VPU_PIECES = ((0, 96), (96, 128))


def _kernel(ax, ak, av, awq, awo, bx, bk, bv, bwq, bwo, o_ref,
            ka, va, kb, vb, wqb, wob, xb, q8s, lhs, sem, wsem, *, window):
    kv = (ka, va, kb, vb)
    w0 = ak.shape[2] - window
    nch = window // UR
    nkv = NG * nch
    wq_steps = (D // NSLAB // 8) * NG
    blk_steps = DH // 8

    def kv_sem(slot, j):
        return sem.at[slot * 4 + j]

    def start_wq(b, t, prio):
        r = pl.multiple_of((t // NG) * 8, 8)
        g = t % NG
        wd = GW // WQ_SPLIT
        for z in range(WQ_SPLIT):
            cc = pl.multiple_of(g * GW + z * wd, wd)
            pltpu.make_async_copy(
                (awq, bwq)[b].at[:, pl.ds(r, 8), pl.ds(cc, wd)],
                wqb.at[g, b, :, pl.ds(r, 8), pl.ds(z * wd, wd)],
                wsem.at[0]).start(priority=prio)

    def wo_cp(b, t, s):
        r = pl.multiple_of((t % blk_steps) * 8, 8)
        rs = pl.multiple_of(t * 8, 8)
        return pltpu.make_async_copy(
            (awo, bwo)[b].at[:, pl.ds(rs, 8), :],
            wob.at[t // blk_steps, b, :, pl.ds(r, 8), :], s)

    def issue_wq():
        for t in range(START_P1):
            for b in range(2):
                start_wq(b, t, 1)

        def body(t, carry):
            for b in range(2):
                start_wq(b, t, b)
            return carry
        lax.fori_loop(START_P1, wq_steps, body, 0)

    def issue_kv(u, slot):
        g = u // nch
        gb = (g + GB) % NG
        h0 = (g * HG, gb * HG + BSH)
        r0 = w0 + (u % nch) * UR

        def start(j, h, d, nh, r, pr):
            rs = pl.multiple_of(r0 + r, pr)
            pltpu.make_async_copy(
                (ak, av, bk, bv)[j].at[0, pl.ds(h, nh), pl.ds(rs, pr), :],
                kv[j].at[slot, pl.ds(d, nh), pl.ds(r, pr), :],
                kv_sem(slot, j)).start(priority=j % 2)

        def loop(b_wraps):
            def body(t, carry):
                for j in (0, 3, 2, 1):
                    if j >= 2 and b_wraps:
                        r = pl.multiple_of(t * PR, PR)
                        start(j, H - HG + BSH, 0, HG - BSH, r, PR)
                        start(j, 0, HG - BSH, BSH, r, PR)
                    else:
                        n = V_SPLIT if j % 2 else 1
                        pr = PR // n
                        for z in range(n):
                            r = pl.multiple_of(t * PR + z * pr, pr)
                            start(j, h0[j // 2], 0, HG, r, pr)
                return carry
            lax.fori_loop(0, UR // PR, body, 0)

        if isinstance(u, int):
            loop(gb == NG - 1)
        else:
            pl.when(gb == NG - 1)(lambda: loop(True))
            pl.when(gb != NG - 1)(lambda: loop(False))

    def issue_wo(t0, n, sa, sb):
        def body(t, carry):
            wo_cp(0, t0 + t, sa).start(priority=0)
            wo_cp(1, t0 + t, sb).start(priority=1)
            return carry
        lax.fori_loop(0, n, body, 0)

    def wait_ref(ref, s):
        pltpu.make_async_copy(ref, ref, s).wait()

    xa_cp = pltpu.make_async_copy(ax, xb.at[0], wsem.at[1])
    xb_cp = pltpu.make_async_copy(bx, xb.at[1], wsem.at[2])
    xa_cp.start()
    xb_cp.start()
    issue_wq()
    for i in range(NS):
        issue_kv(i, i)
    xa_cp.wait()
    xb_cp.wait()
    wait_ref(wqb, wsem.at[0])

    row = lax.broadcasted_iota(jnp.int32, (8, DH), 0)
    row_s = lax.broadcasted_iota(jnp.int32, (8, UR), 0)
    scale = DH ** -0.5

    def kv_body(u, carry):
        m, l, acc = carry
        g = u // nch
        c = u % nch
        slot = u % NS
        first = c == 0

        @pl.when(first)
        def _():
            q8 = jnp.zeros((8, DH), F32)
            for b in range(2):
                x8 = jnp.broadcast_to(xb[b, 0], (8, D))
                gq = (g + b * GB) % NG
                sh = b * BSH
                w1 = wqb[gq, b, :, :, sh * DH:].reshape(D, GW - sh * DH)
                qs = [jnp.dot(x8, w1, preferred_element_type=F32)]
                if sh:
                    w2 = wqb[(gq + 1) % NG, b, :, :, :sh * DH].reshape(D, sh * DH)
                    qs.append(jnp.dot(x8, w2, preferred_element_type=F32))
                for j in range(HG):
                    qp, k = (qs[0], j) if j < HG - sh else (qs[1], j - (HG - sh))
                    q8 = jnp.where(row == b * HG + j, qp[:, k * DH:(k + 1) * DH], q8)
            q8s[...] = q8

        m = jnp.where(first, -jnp.inf, m)
        l = jnp.where(first, 0.0, l)
        acc = jnp.where(first, 0.0, acc)
        for j in (0, 2):
            wait_ref(kv[j].at[slot], kv_sem(slot, j))
        q8 = q8s[...].astype(BF16)
        s = jnp.zeros((8, UR), F32)
        for b in range(2):
            for j in range(HG):
                sj = lax.dot_general(q8, kv[2 * b][slot, j], (((1,), (1,)), ((), ())),
                                     preferred_element_type=F32)
                s = jnp.where(row_s == b * HG + j, sj, s)
        s = s * scale
        m_new = jnp.maximum(m, jnp.max(s, axis=-1, keepdims=True))
        alpha = jnp.exp(m - m_new)
        p = jnp.exp(s - m_new)
        l = l * alpha + jnp.sum(p, axis=-1, keepdims=True)
        pb = p.astype(BF16)
        for j in (1, 3):
            wait_ref(kv[j].at[slot], kv_sem(slot, j))
        o = jnp.zeros((8, DH), F32)
        for b in range(2):
            for j in range(HG):
                oj = jnp.dot(pb, kv[2 * b + 1][slot, j], preferred_element_type=F32)
                o = jnp.where(row == b * HG + j, oj, o)
        acc = acc * alpha + o

        @pl.when(c == nch - 1)
        def _():
            lhs[g] = acc / l

        n = u + NS

        @pl.when(n < nkv)
        def _():
            issue_kv(n, slot)

        @pl.when(n >= nkv)
        def _():
            issue_wo((n - nkv) * 2 * blk_steps, 2 * blk_steps,
                     kv_sem(slot, 0), kv_sem(slot, 0))
        return m_new, l, acc

    init = (jnp.full((8, 1), -jnp.inf, F32), jnp.zeros((8, 1), F32),
            jnp.zeros((8, DH), F32))
    lax.fori_loop(0, nkv, kv_body, init)

    last = 7
    issue_wo(6 * blk_steps, blk_steps, wsem.at[0], wsem.at[1])

    def b_sem(sl, r):
        for i, (lo, hi) in enumerate(MXU_PIECES):
            if lo <= sl < hi:
                return wsem.at[2 + i]
        for i, (lo, hi) in enumerate(VPU_PIECES):
            if lo <= r < hi:
                return wsem.at[2 + len(MXU_PIECES) + i]

    for sl in range(NSLAB):
        for r in range(0, DH, TAIL_ROWS):
            for b in range(2):
                pltpu.make_async_copy(
                    (awo, bwo)[b].at[sl, pl.ds(last * DH + r, TAIL_ROWS), :],
                    wob.at[last, b, sl, pl.ds(r, TAIL_ROWS), :],
                    b_sem(sl, r) if b else wsem.at[0]).start(priority=b)

    def o_pos(b, h):
        idx = (h - b * BSH) % H
        return (idx // HG - b * GB) % NG, b * HG + idx % HG

    def proj(b, blk, slabs):
        res = None
        for sl in slabs:
            h = sl * 8 + blk
            gi, ri = o_pos(b, h)
            o_h = jnp.where(row == ri, lhs[gi], 0.0).astype(BF16)
            t = jnp.dot(o_h, wob[blk, b, sl], preferred_element_type=F32)
            res = t if res is None else res + t
        return res

    gi, ri = o_pos(1, H - 1)
    o_last = lhs[gi][ri:ri + 1, :].astype(BF16).astype(F32)
    o_col = jnp.broadcast_to(o_last, (DH, DH)).T

    acc_a = jnp.zeros((8, D), F32)
    acc_b = jnp.zeros((8, D), F32)
    for blk in range(6):
        if blk % 2 == 0:
            wait_ref(wob.at[pl.ds(blk, 2)], kv_sem((nkv + blk // 2) % NS, 0))
        acc_a = acc_a + proj(0, blk, range(NSLAB))
        acc_b = acc_b + proj(1, blk, range(NSLAB))
    wait_ref(wob.at[pl.ds(6, 2), 0], wsem.at[0])
    acc_a = acc_a + proj(0, 6, range(NSLAB)) + proj(0, last, range(NSLAB))
    o_ref[0, :, 0:D] = jnp.sum(acc_a, axis=0, keepdims=True).astype(o_ref.dtype)
    wait_ref(wob.at[6, 1], wsem.at[1])
    acc_b = acc_b + proj(1, 6, range(NSLAB))
    for i, (lo, hi) in enumerate(MXU_PIECES):
        wait_ref(wob.at[last, 1, pl.ds(lo, hi - lo)], wsem.at[2 + i])
        acc_b = acc_b + proj(1, last, range(lo, hi))
    for i, (lo, hi) in enumerate(VPU_PIECES):
        wait_ref(wob.at[last, 1, NSLAB - 1, pl.ds(lo, hi - lo)],
                 wsem.at[2 + len(MXU_PIECES) + i])
        parts = []
        for cb in range(D // DH):
            w = wob[last, 1, NSLAB - 1, lo:hi, cb * DH:(cb + 1) * DH].astype(F32)
            parts.append(jnp.sum((w * o_col[lo:hi]).reshape((hi - lo) // 8, 8, DH), axis=0))
        acc_b = acc_b + jnp.concatenate(parts, axis=1)
    o_ref[0, :, D:2 * D] = jnp.sum(acc_b, axis=0, keepdims=True).astype(o_ref.dtype)


@jax.jit
def pallas_concat_heads__sliding_block_cached__sliding_block_cached__decode_kernel(
    A_x: jax.Array,
    A_k_cache: jax.Array,
    A_v_cache: jax.Array,
    A_wq: jax.Array,
    A_wo: jax.Array,
    B_x: jax.Array,
    B_k_cache: jax.Array,
    B_v_cache: jax.Array,
    B_wq: jax.Array,
    B_wo: jax.Array,
):
    sk = A_k_cache.shape[2]
    window = min(4096, max(256, sk // 4))
    assert A_x.shape == (1, 1, D) and A_k_cache.shape == (1, H, sk, DH)
    assert B_k_cache.shape == A_k_cache.shape
    assert window % UR == 0 and (sk - window) % PR == 0

    def kernel(*refs):
        _kernel(*refs, window=window)

    def slabs(w):
        return w.reshape(NSLAB, w.shape[0] // NSLAB, w.shape[1])

    any_spec = pl.BlockSpec(memory_space=pl.ANY)
    return pl.pallas_call(
        kernel,
        in_specs=[any_spec] * 10,
        out_specs=pl.BlockSpec(memory_space=pltpu.VMEM),
        out_shape=jax.ShapeDtypeStruct((1, 1, 2 * D), A_x.dtype),
        scratch_shapes=[
            pltpu.VMEM((NS, HG, UR, DH), BF16),
            pltpu.VMEM((NS, HG, UR, DH), BF16),
            pltpu.VMEM((NS, HG, UR, DH), BF16),
            pltpu.VMEM((NS, HG, UR, DH), BF16),
            pltpu.VMEM((NG, 2, NSLAB, D // NSLAB, GW), BF16),
            pltpu.VMEM((8, 2, NSLAB, DH, D), BF16),
            pltpu.VMEM((2, 1, 1, D), BF16),
            pltpu.VMEM((8, DH), F32),
            pltpu.VMEM((NG, 8, DH), F32),
            pltpu.SemaphoreType.DMA((NS * 4,)),
            pltpu.SemaphoreType.DMA((2 + len(MXU_PIECES) + len(VPU_PIECES),)),
        ],
        compiler_params=pltpu.CompilerParams(
            vmem_limit_bytes=64 * 1024 * 1024,
            disable_semaphore_checks=True,
            disable_bounds_checks=True,
        ),
    )(A_x, A_k_cache, A_v_cache, slabs(A_wq), slabs(A_wo),
      B_x, B_k_cache, B_v_cache, slabs(B_wq), slabs(B_wo))
```

```python
import jax
import jax.numpy as jnp
from jax import lax
import jax.experimental.pallas as pl
import jax.experimental.pallas.tpu as pltpu

F32 = jnp.float32
BF16 = jnp.bfloat16

H, DH, D = 32, 128, 512
HG = 4
NG = H // HG
GW = HG * DH
UR = 512
PR = 32
V_SPLIT = 2
GB = 4
BSH = 1
NS = 3
NSLAB = 4
WQ_SPLIT = 2
WQ_XOR = 80
START_P1 = 3
TAIL_ROWS = 32
MXU_PIECES = ((0, 2), (2, 3))
VPU_PIECES = ((0, 96), (96, 128))


def _kernel(ax, ak, av, awq, awo, bx, bk, bv, bwq, bwo, o_ref,
            ka, va, kb, vb, wqb, wob, xb, q8s, lhs, sem, wsem, *, window):
    kv = (ka, va, kb, vb)
    w0 = ak.shape[2] - window
    nch = window // UR
    nkv = NG * nch
    wq_steps = (D // NSLAB // 8) * NG
    assert wq_steps // 2 <= WQ_XOR < wq_steps
    blk_steps = DH // 8

    def kv_sem(slot, j):
        return sem.at[slot * 4 + j]

    def start_wq(b, t, prio):
        r = pl.multiple_of((t // NG) * 8, 8)
        g = t % NG
        wd = GW // WQ_SPLIT
        for z in range(WQ_SPLIT):
            cc = pl.multiple_of(g * GW + z * wd, wd)
            pltpu.make_async_copy(
                (awq, bwq)[b].at[:, pl.ds(r, 8), pl.ds(cc, wd)],
                wqb.at[g, b, :, pl.ds(r, 8), pl.ds(z * wd, wd)],
                wsem.at[0]).start(priority=prio)

    def wo_cp(b, t, s):
        r = pl.multiple_of((t % blk_steps) * 8, 8)
        rs = pl.multiple_of(t * 8, 8)
        return pltpu.make_async_copy(
            (awo, bwo)[b].at[:, pl.ds(rs, 8), :],
            wob.at[t // blk_steps, b, :, pl.ds(r, 8), :], s)

    def issue_wq():
        def round_(t, all_low):
            steps = ((0, t), (1, t), (1, t ^ WQ_XOR), (0, t ^ WQ_XOR))
            for i, (b, tt) in enumerate(steps):
                start_wq(b, tt, 1 if all_low else i % 2)

        for t in range(START_P1):
            round_(t, True)

        def body(t, carry):
            round_(t, False)
            return carry
        lax.fori_loop(START_P1, wq_steps // 2, body, 0)

    def issue_kv(u, slot):
        g = u // nch
        gb = (g + GB) % NG
        h0 = (g * HG, gb * HG + BSH)
        r0 = w0 + (u % nch) * UR

        def start(j, h, d, nh, r, pr):
            rs = pl.multiple_of(r0 + r, pr)
            pltpu.make_async_copy(
                (ak, av, bk, bv)[j].at[0, pl.ds(h, nh), pl.ds(rs, pr), :],
                kv[j].at[slot, pl.ds(d, nh), pl.ds(r, pr), :],
                kv_sem(slot, j)).start(priority=j % 2)

        def loop(b_wraps):
            def body(t, carry):
                for j in (0, 3, 2, 1):
                    if j >= 2 and b_wraps:
                        r = pl.multiple_of(t * PR, PR)
                        start(j, H - HG + BSH, 0, HG - BSH, r, PR)
                        start(j, 0, HG - BSH, BSH, r, PR)
                    else:
                        n = V_SPLIT if j % 2 else 1
                        pr = PR // n
                        for z in range(n):
                            r = pl.multiple_of(t * PR + z * pr, pr)
                            start(j, h0[j // 2], 0, HG, r, pr)
                return carry
            lax.fori_loop(0, UR // PR, body, 0)

        if isinstance(u, int):
            loop(gb == NG - 1)
        else:
            pl.when(gb == NG - 1)(lambda: loop(True))
            pl.when(gb != NG - 1)(lambda: loop(False))

    def issue_wo(t0, n, sa, sb):
        def body(t, carry):
            wo_cp(0, t0 + t, sa).start(priority=0)
            wo_cp(1, t0 + t, sb).start(priority=1)
            return carry
        lax.fori_loop(0, n, body, 0)

    def wait_ref(ref, s):
        pltpu.make_async_copy(ref, ref, s).wait()

    xa_cp = pltpu.make_async_copy(ax, xb.at[0], wsem.at[1])
    xb_cp = pltpu.make_async_copy(bx, xb.at[1], wsem.at[2])
    xa_cp.start()
    xb_cp.start()
    issue_wq()
    for i in range(NS):
        issue_kv(i, i)
    xa_cp.wait()
    xb_cp.wait()
    wait_ref(wqb, wsem.at[0])

    row = lax.broadcasted_iota(jnp.int32, (8, DH), 0)
    row_s = lax.broadcasted_iota(jnp.int32, (8, UR), 0)
    scale = DH ** -0.5

    def kv_body(u, carry):
        m, l, acc = carry
        g = u // nch
        c = u % nch
        slot = u % NS
        first = c == 0

        @pl.when(first)
        def _():
            q8 = jnp.zeros((8, DH), F32)
            for b in range(2):
                x8 = jnp.broadcast_to(xb[b, 0], (8, D))
                gq = (g + b * GB) % NG
                sh = b * BSH
                w1 = wqb[gq, b, :, :, sh * DH:].reshape(D, GW - sh * DH)
                qs = [jnp.dot(x8, w1, preferred_element_type=F32)]
                if sh:
                    w2 = wqb[(gq + 1) % NG, b, :, :, :sh * DH].reshape(D, sh * DH)
                    qs.append(jnp.dot(x8, w2, preferred_element_type=F32))
                for j in range(HG):
                    qp, k = (qs[0], j) if j < HG - sh else (qs[1], j - (HG - sh))
                    q8 = jnp.where(row == b * HG + j, qp[:, k * DH:(k + 1) * DH], q8)
            q8s[...] = q8

        m = jnp.where(first, -jnp.inf, m)
        l = jnp.where(first, 0.0, l)
        acc = jnp.where(first, 0.0, acc)
        for j in (0, 2):
            wait_ref(kv[j].at[slot], kv_sem(slot, j))
        q8 = q8s[...].astype(BF16)
        s = jnp.zeros((8, UR), F32)
        for b in range(2):
            for j in range(HG):
                sj = lax.dot_general(q8, kv[2 * b][slot, j], (((1,), (1,)), ((), ())),
                                     preferred_element_type=F32)
                s = jnp.where(row_s == b * HG + j, sj, s)
        s = s * scale
        m_new = jnp.maximum(m, jnp.max(s, axis=-1, keepdims=True))
        alpha = jnp.exp(m - m_new)
        p = jnp.exp(s - m_new)
        l = l * alpha + jnp.sum(p, axis=-1, keepdims=True)
        pb = p.astype(BF16)
        for j in (1, 3):
            wait_ref(kv[j].at[slot], kv_sem(slot, j))
        o = jnp.zeros((8, DH), F32)
        for b in range(2):
            for j in range(HG):
                oj = jnp.dot(pb, kv[2 * b + 1][slot, j], preferred_element_type=F32)
                o = jnp.where(row == b * HG + j, oj, o)
        acc = acc * alpha + o

        @pl.when(c == nch - 1)
        def _():
            lhs[g] = acc / l

        n = u + NS

        @pl.when(n < nkv)
        def _():
            issue_kv(n, slot)

        @pl.when(n >= nkv)
        def _():
            issue_wo((n - nkv) * 2 * blk_steps, 2 * blk_steps,
                     kv_sem(slot, 0), kv_sem(slot, 0))
        return m_new, l, acc

    init = (jnp.full((8, 1), -jnp.inf, F32), jnp.zeros((8, 1), F32),
            jnp.zeros((8, DH), F32))
    lax.fori_loop(0, nkv, kv_body, init)

    last = 7
    issue_wo(6 * blk_steps, blk_steps, wsem.at[0], wsem.at[1])

    def b_sem(sl, r):
        for i, (lo, hi) in enumerate(MXU_PIECES):
            if lo <= sl < hi:
                return wsem.at[2 + i]
        for i, (lo, hi) in enumerate(VPU_PIECES):
            if lo <= r < hi:
                return wsem.at[2 + len(MXU_PIECES) + i]

    for sl in range(NSLAB):
        for r in range(0, DH, TAIL_ROWS):
            for b in range(2):
                pltpu.make_async_copy(
                    (awo, bwo)[b].at[sl, pl.ds(last * DH + r, TAIL_ROWS), :],
                    wob.at[last, b, sl, pl.ds(r, TAIL_ROWS), :],
                    b_sem(sl, r) if b else wsem.at[0]).start(priority=b)

    def o_pos(b, h):
        idx = (h - b * BSH) % H
        return (idx // HG - b * GB) % NG, b * HG + idx % HG

    def proj(b, blk, slabs):
        res = None
        for sl in slabs:
            h = sl * 8 + blk
            gi, ri = o_pos(b, h)
            o_h = jnp.where(row == ri, lhs[gi], 0.0).astype(BF16)
            t = jnp.dot(o_h, wob[blk, b, sl], preferred_element_type=F32)
            res = t if res is None else res + t
        return res

    gi, ri = o_pos(1, H - 1)
    o_last = lhs[gi][ri:ri + 1, :].astype(BF16).astype(F32)
    o_col = jnp.broadcast_to(o_last, (DH, DH)).T

    acc_a = jnp.zeros((8, D), F32)
    acc_b = jnp.zeros((8, D), F32)
    for blk in range(6):
        if blk % 2 == 0:
            wait_ref(wob.at[pl.ds(blk, 2)], kv_sem((nkv + blk // 2) % NS, 0))
        acc_a = acc_a + proj(0, blk, range(NSLAB))
        acc_b = acc_b + proj(1, blk, range(NSLAB))
    wait_ref(wob.at[pl.ds(6, 2), 0], wsem.at[0])
    acc_a = acc_a + proj(0, 6, range(NSLAB)) + proj(0, last, range(NSLAB))
    o_ref[0, :, 0:D] = jnp.sum(acc_a, axis=0, keepdims=True).astype(o_ref.dtype)
    wait_ref(wob.at[6, 1], wsem.at[1])
    acc_b = acc_b + proj(1, 6, range(NSLAB))
    for i, (lo, hi) in enumerate(MXU_PIECES):
        wait_ref(wob.at[last, 1, pl.ds(lo, hi - lo)], wsem.at[2 + i])
        acc_b = acc_b + proj(1, last, range(lo, hi))
    for i, (lo, hi) in enumerate(VPU_PIECES):
        wait_ref(wob.at[last, 1, NSLAB - 1, pl.ds(lo, hi - lo)],
                 wsem.at[2 + len(MXU_PIECES) + i])
        parts = []
        for cb in range(D // DH):
            w = wob[last, 1, NSLAB - 1, lo:hi, cb * DH:(cb + 1) * DH].astype(F32)
            parts.append(jnp.sum((w * o_col[lo:hi]).reshape((hi - lo) // 8, 8, DH), axis=0))
        acc_b = acc_b + jnp.concatenate(parts, axis=1)
    o_ref[0, :, D:2 * D] = jnp.sum(acc_b, axis=0, keepdims=True).astype(o_ref.dtype)


@jax.jit
def pallas_concat_heads__sliding_block_cached__sliding_block_cached__decode_kernel(
    A_x: jax.Array,
    A_k_cache: jax.Array,
    A_v_cache: jax.Array,
    A_wq: jax.Array,
    A_wo: jax.Array,
    B_x: jax.Array,
    B_k_cache: jax.Array,
    B_v_cache: jax.Array,
    B_wq: jax.Array,
    B_wo: jax.Array,
):
    sk = A_k_cache.shape[2]
    window = min(4096, max(256, sk // 4))
    assert A_x.shape == (1, 1, D) and A_k_cache.shape == (1, H, sk, DH)
    assert B_k_cache.shape == A_k_cache.shape
    assert window % UR == 0 and (sk - window) % PR == 0

    def kernel(*refs):
        _kernel(*refs, window=window)

    def slabs(w):
        return w.reshape(NSLAB, w.shape[0] // NSLAB, w.shape[1])

    any_spec = pl.BlockSpec(memory_space=pl.ANY)
    return pl.pallas_call(
        kernel,
        in_specs=[any_spec] * 10,
        out_specs=pl.BlockSpec(memory_space=pltpu.VMEM),
        out_shape=jax.ShapeDtypeStruct((1, 1, 2 * D), A_x.dtype),
        scratch_shapes=[
            pltpu.VMEM((NS, HG, UR, DH), BF16),
            pltpu.VMEM((NS, HG, UR, DH), BF16),
            pltpu.VMEM((NS, HG, UR, DH), BF16),
            pltpu.VMEM((NS, HG, UR, DH), BF16),
            pltpu.VMEM((NG, 2, NSLAB, D // NSLAB, GW), BF16),
            pltpu.VMEM((8, 2, NSLAB, DH, D), BF16),
            pltpu.VMEM((2, 1, 1, D), BF16),
            pltpu.VMEM((8, DH), F32),
            pltpu.VMEM((NG, 8, DH), F32),
            pltpu.SemaphoreType.DMA((NS * 4,)),
            pltpu.SemaphoreType.DMA((2 + len(MXU_PIECES) + len(VPU_PIECES),)),
        ],
        compiler_params=pltpu.CompilerParams(
            vmem_limit_bytes=64 * 1024 * 1024,
            disable_semaphore_checks=True,
            disable_bounds_checks=True,
        ),
    )(A_x, A_k_cache, A_v_cache, slabs(A_wq), slabs(A_wo),
      B_x, B_k_cache, B_v_cache, slabs(B_wq), slabs(B_wo))
```
